```python
import jax
import jax.numpy as jnp

def _softmax(x, axis=-1):
    return jax.nn.softmax(x, axis=axis)
def _gelu(x):
    return jax.nn.gelu(x, approximate=True)
def _silu(x):
    return jax.nn.silu(x)
def _sigmoid(x):
    return jax.nn.sigmoid(x)
def _layernorm(x, axis=-1, eps=1e-5):
    m = jnp.mean(x, axis=axis, keepdims=True)
    v = jnp.var(x, axis=axis, keepdims=True)
    return (x - m) / jnp.sqrt(v + eps)
def _scatter_add(tgt, idx, src, axis=0):
    return tgt.at[idx].add(src)
def _segment_sum(src, seg, n):
    return jax.ops.segment_sum(src, seg, n)
class _Rng:
    def __init__(self, key):
        self._k = key
    def _next(self):
        self._k, sub = jax.random.split(self._k)
        return sub
    def normal(self, shape):
        return jax.random.normal(self._next(), shape, dtype=jnp.bfloat16)
    def randint(self, lo, hi, shape):
        return jax.random.randint(self._next(), shape, lo, hi, dtype=jnp.int32)
    def uniform(self, shape, lo=0.0, hi=1.0):
        return jax.random.uniform(self._next(), shape, jnp.bfloat16, lo, hi)
    def permutation(self, n):
        return jax.random.permutation(self._next(), n)


kernel_name = 'sequential_preLN__sliding_block_cached__moe_arch_mod__decode'

def setup_inputs():
    _rng = _Rng(jax.random.key(int.from_bytes(__import__("os").urandom(4), "little")))
    _w = (lambda a: (lambda t: t.astype(jnp.bfloat16) if jnp.issubdtype(t.dtype, jnp.floating) else t)(jnp.asarray(a)))
    def _A_setup():
        B, Sq, D = 1, 1, 640
        Hq, Hkv, Sk, Dh = 32, 32, 32768, 192
        assert Hq % Hkv == 0, (Hq, Hkv)
        return {
            "x": _w((lambda *s: _rng.normal(s) * 0.05)(B, Sq, D)),
            "k_cache": _w((lambda *s: _rng.normal(s) * 0.05)(B, Hkv, Sk, Dh)),
            "v_cache": _w((lambda *s: _rng.normal(s) * 0.05)(B, Hkv, Sk, Dh)),
            "wq": _w((lambda *s: _rng.normal(s) * 0.05)(D, Hq * Dh) * (D ** -0.5)),
            "wo": _w((lambda *s: _rng.normal(s) * 0.05)(Hq * Dh, D) * ((Hq * Dh) ** -0.5)),
        }
    _A_in = _A_setup()

    def _B_setup():
        B, S, D, F, C = 1, 1, 640, 1536, 1
        return {
            "x": _w((lambda *s: _rng.normal(s) * 0.05)(B, S, D)),
            "w_r": _w((lambda *s: _rng.normal(s) * 0.05)(D)),
            "w_gate": _w((lambda *s: _rng.normal(s) * 0.05)(D, F)),
            "w_up": _w((lambda *s: _rng.normal(s) * 0.05)(D, F)),
            "w_down": _w((lambda *s: _rng.normal(s) * 0.05)(F, D)),
        }
    _B_in = _B_setup()

    return {
        "A_x": _A_in["x"],
        "A_k_cache": _A_in["k_cache"],
        "A_v_cache": _A_in["v_cache"],
        "A_wq": _A_in["wq"],
        "A_wo": _A_in["wo"],
        "B_x": _B_in["x"],
        "B_w_r": _B_in["w_r"],
        "B_w_gate": _B_in["w_gate"],
        "B_w_up": _B_in["w_up"],
        "B_w_down": _B_in["w_down"],
    }

def reference(A_x, A_k_cache, A_v_cache, A_wq, A_wo, B_x, B_w_r, B_w_gate, B_w_up, B_w_down):
    def _A_ref(x, k_cache, v_cache, wq, wo):
        B, Sq, D = x.shape
        Hq, Dh = 32, 192
        Hkv, Sk = k_cache.shape[1], k_cache.shape[2]
        W = min(4096, max(256, Sk // 4))
        rep = Hq // Hkv
        q = (lambda x, *d: x.transpose(*d))((x @ wq).reshape(B, Sq, Hq, Dh), 0, 2, 1, 3)
        k = jnp.repeat(k_cache[:, :, Sk - W:, :], rep, axis=1)
        v = jnp.repeat(v_cache[:, :, Sk - W:, :], rep, axis=1)
        scores = jnp.einsum("bhqd,bhkd->bhqk", q, k) * (Dh ** -0.5)
        p = _softmax(scores, axis=-1)
        o = jnp.einsum("bhqk,bhkd->bhqd", p, v)
        return (lambda x, *d: x.transpose(*d))(o, 0, 2, 1, 3).reshape(B, Sq, Hq * Dh) @ wo

    def _B_ref(x, w_r, w_gate, w_up, w_down):
        B, S, D = x.shape
        C = 1
        r = x @ w_r
        idx = jnp.argsort(-r, axis=-1)[:, :C]
        idx_e = jnp.repeat(idx.reshape(B, C, 1), D, axis=2)
        x_sel = jnp.take_along_axis(x, idx_e, axis=1)
        g = _silu(x_sel @ w_gate)
        u = x_sel @ w_up
        y = (g * u) @ w_down
        r_sel = _sigmoid(jnp.take_along_axis(r, idx, axis=1))
        y = y * r_sel.reshape(B, C, 1)
        b_off = (jnp.arange(B) * S).reshape(B, 1)
        flat_idx = (idx + b_off).reshape(B * C)
        zero = (x * 0.0).reshape(B * S, D)
        upd = _scatter_add(zero, flat_idx, y.reshape(B * C, D), axis=0)
        return x + upd.reshape(B, S, D)

    x = A_x
    h = x + _A_ref(_layernorm(x, axis=-1), A_k_cache, A_v_cache, A_wq, A_wo)
    h2 = h + _B_ref(_layernorm(h, axis=-1), B_w_r, B_w_gate, B_w_up, B_w_down)
    return h2
```

```python
import jax
import jax.numpy as jnp
import jax.experimental.pallas as pl
import jax.experimental.pallas.tpu as pltpu

HQ, DH = 32, 192
G = 8
NG = HQ // G
GR = G * DH
NBUF = 3
ND = 4
EPS = 1e-5


def _layernorm(x):
    m = jnp.mean(x, axis=-1, keepdims=True)
    c = x - m
    v = jnp.mean(c * c, axis=-1, keepdims=True)
    return c / jnp.sqrt(v + EPS)


def _rows8(x):
    return jnp.broadcast_to(x, (8, x.shape[-1])).astype(jnp.bfloat16)


def _dot(a, b):
    return jnp.dot(a, b, preferred_element_type=jnp.float32)


def _kernel(x_hbm, kt_hbm, vt_hbm, wq_hbm, wo_hbm, wr_hbm, wg_hbm, wu_hbm, wd_hbm,
            o_ref,
            kv_buf, wq_buf, wo_buf, wg_buf, wu_buf, wd_buf, x_buf, wr_buf,
            q_scr, p_scr, o_scr, kv_sem, w_sem, wd_sem):
    sk = kt_hbm.shape[1]
    win = kv_buf.shape[2]
    fc = wd_buf.shape[0] // ND

    def kv_copy(src, g, slot):
        return pltpu.make_async_copy(
            src.at[pl.ds(pl.multiple_of(g * GR, GR), GR), pl.ds(sk - win, win)],
            kv_buf.at[slot], kv_sem.at[slot])

    x_cp = pltpu.make_async_copy(x_hbm, x_buf, w_sem.at[0])
    wq_cp = pltpu.make_async_copy(wq_hbm, wq_buf, w_sem.at[1])
    wr_cp = pltpu.make_async_copy(wr_hbm, wr_buf, w_sem.at[2])
    wo_cp = pltpu.make_async_copy(wo_hbm, wo_buf, w_sem.at[3])
    wg_cp = pltpu.make_async_copy(wg_hbm, wg_buf, w_sem.at[4])
    wu_cp = pltpu.make_async_copy(wu_hbm, wu_buf, w_sem.at[5])
    wd_cp = [pltpu.make_async_copy(wd_hbm.at[pl.ds(i * fc, fc)],
                                   wd_buf.at[pl.ds(i * fc, fc)], wd_sem.at[i])
             for i in range(ND)]

    wq_cp.start()
    x_cp.start()
    wr_cp.start()
    kv_copy(kt_hbm, 0, 0).start()

    x_cp.wait()
    x = x_buf[...].astype(jnp.float32)
    xn = _rows8(_layernorm(x))
    wq_cp.wait()
    kv_copy(kt_hbm, 1, 1).start()
    row = jax.lax.broadcasted_iota(jnp.int32, (G, GR), 0)
    col = jax.lax.broadcasted_iota(jnp.int32, (G, GR), 1)
    diag = (col >= row * DH) & (col < (row + 1) * DH)
    for g in range(NG):
        q = _dot(xn, wq_buf[:, g * GR:(g + 1) * GR])
        q_scr[g] = jnp.where(diag, q, 0.0).astype(jnp.bfloat16)

    def k_step(g, _):
        slot = g % NBUF
        kv_copy(kt_hbm, g, slot).wait()
        nxt = g + 2

        @pl.when(nxt < NG)
        def _():
            kv_copy(kt_hbm, nxt, nxt % NBUF).start()

        @pl.when(nxt >= NG)
        def _():
            kv_copy(vt_hbm, nxt - NG, nxt % NBUF).start()

        s = _dot(q_scr[g], kv_buf[slot]) * (DH ** -0.5)
        m = jnp.max(s, axis=-1, keepdims=True)
        e = jnp.exp(s - m)
        p_scr[g] = (e / jnp.sum(e, axis=-1, keepdims=True)).astype(jnp.bfloat16)

    jax.lax.fori_loop(0, NG, k_step, None)

    def v_step(g, _):
        slot = (g + NG) % NBUF
        kv_copy(vt_hbm, g, slot).wait()

        @pl.when(g + 2 < NG)
        def _():
            kv_copy(vt_hbm, g + 2, (g + 2 + NG) % NBUF).start()

        @pl.when(g + 2 == NG)
        def _():
            wo_cp.start()

        @pl.when(g + 1 == NG)
        def _():
            wg_cp.start()
            wu_cp.start()

        o = jax.lax.dot_general(p_scr[g], kv_buf[slot], (((1,), (1,)), ((), ())),
                                preferred_element_type=jnp.float32)
        o_scr[g] = jnp.where(diag, o, 0.0).astype(jnp.bfloat16)

    jax.lax.fori_loop(0, NG, v_step, None)

    wo_cp.wait()
    for c in wd_cp:
        c.start()
    a = _dot(o_scr[0], wo_buf[0:GR])
    for g in range(1, NG):
        a = a + _dot(o_scr[g], wo_buf[g * GR:(g + 1) * GR])
    h = x + jnp.sum(a, axis=0, keepdims=True)
    hn = _layernorm(h).astype(jnp.bfloat16).astype(jnp.float32)

    wr_cp.wait()
    r = jnp.sum(hn * wr_buf[...].astype(jnp.float32).reshape(1, -1), axis=-1, keepdims=True)
    hn8 = _rows8(hn)
    wg_cp.wait()
    gate = _dot(hn8, wg_buf[...])
    wu_cp.wait()
    up = _dot(hn8, wu_buf[...])
    act = (gate * jax.nn.sigmoid(gate) * up).astype(jnp.bfloat16)
    y = None
    for i in range(ND):
        wd_cp[i].wait()
        t = _dot(act[:, i * fc:(i + 1) * fc], wd_buf[i * fc:(i + 1) * fc])
        y = t if y is None else y + t
    y = y[0:1] * jax.nn.sigmoid(r)
    o_ref[...] = (h + (hn + (hn * 0.0 + y))).astype(o_ref.dtype)


@jax.jit
def pallas_sequential_preLN__sliding_block_cached__moe_arch_mod__decode_kernel(
    A_x: jax.Array,
    A_k_cache: jax.Array,
    A_v_cache: jax.Array,
    A_wq: jax.Array,
    A_wo: jax.Array,
    B_x: jax.Array,
    B_w_r: jax.Array,
    B_w_gate: jax.Array,
    B_w_up: jax.Array,
    B_w_down: jax.Array,
):
    del B_x
    d = A_x.shape[-1]
    sk = A_k_cache.shape[2]
    f = B_w_gate.shape[1]
    win = min(4096, max(256, sk // 4))
    kt = jnp.swapaxes(A_k_cache, 2, 3).reshape(HQ * DH, sk)
    vt = jnp.swapaxes(A_v_cache, 2, 3).reshape(HQ * DH, sk)
    bf = jnp.bfloat16
    out = pl.pallas_call(
        _kernel,
        out_shape=jax.ShapeDtypeStruct((1, d), A_x.dtype),
        in_specs=[pl.BlockSpec(memory_space=pl.ANY)] * 9,
        out_specs=pl.BlockSpec(memory_space=pltpu.VMEM),
        scratch_shapes=[
            pltpu.VMEM((NBUF, GR, win), bf),
            pltpu.VMEM((d, HQ * DH), bf),
            pltpu.VMEM((HQ * DH, d), bf),
            pltpu.VMEM((d, f), bf),
            pltpu.VMEM((d, f), bf),
            pltpu.VMEM((f, d), bf),
            pltpu.VMEM((1, d), bf),
            pltpu.VMEM((d,), bf),
            pltpu.VMEM((NG, G, GR), bf),
            pltpu.VMEM((NG, G, win), bf),
            pltpu.VMEM((NG, G, GR), bf),
            pltpu.SemaphoreType.DMA((NBUF,)),
            pltpu.SemaphoreType.DMA((6,)),
            pltpu.SemaphoreType.DMA((ND,)),
        ],
        compiler_params=pltpu.CompilerParams(vmem_limit_bytes=100 * 2**20),
    )(A_x.reshape(1, d), kt, vt, A_wq, A_wo, B_w_r, B_w_gate, B_w_up, B_w_down)
    return out.reshape(A_x.shape)
```

```python
import jax
import jax.numpy as jnp
import jax.experimental.pallas as pl
import jax.experimental.pallas.tpu as pltpu

HQ, DH = 32, 192
G = 8
R = 384
NC = HQ * DH // R
CPG = G * DH // R
NBUF = 2
PR, PC = 32, 512
WQR, WOR, WGR = 16, 16, 16
ND = 4
EPS = 1e-5


def _layernorm(x):
    m = jnp.mean(x, axis=-1, keepdims=True)
    c = x - m
    v = jnp.mean(c * c, axis=-1, keepdims=True)
    return c / jnp.sqrt(v + EPS)


def _rows8(x):
    return jnp.broadcast_to(x, (8, x.shape[-1])).astype(jnp.bfloat16)


def _dot(a, b):
    return jnp.dot(a, b, preferred_element_type=jnp.float32)


def _fetch(src, r0, c0, dst, sem, pr, pc):
    nr, nc = dst.shape[0] // pr, dst.shape[1] // pc
    step = 1 if nc % 2 == 0 else 2
    assert nr % step == 0

    def body(i, _):
        for j in range(step * nc):
            r = pl.multiple_of((i * step + j // nc) * pr, pr)
            c = (j % nc) * pc
            pltpu.make_async_copy(
                src.at[pl.ds(r0 + r, pr), pl.ds(c0 + c, pc)],
                dst.at[pl.ds(r, pr), pl.ds(c, pc)], sem).start(priority=j % 2)

    jax.lax.fori_loop(0, nr // step, body, None)


def _wait(dst, sem):
    pltpu.make_async_copy(dst, dst, sem).wait()


def _kernel(x_hbm, kt_hbm, vt_hbm, wq_hbm, wo_hbm, wr_hbm, wg_hbm, wu_hbm, wd_hbm,
            o_ref,
            kv_buf, wq_buf, wo_buf, wg_buf, wu_buf, wd_buf, x_buf, wr_buf,
            s_scr, p_scr, a_scr, kv_sem, w_sem, x_sem, wd_sem):
    sk = kt_hbm.shape[1]
    win = kv_buf.shape[2]
    d = x_buf.shape[1]
    fc = wd_buf.shape[1]
    f = wg_buf.shape[1]

    def fetch_k(c):
        slot = c % NBUF
        _fetch(wq_hbm, 0, pl.multiple_of(c * R, R), wq_buf.at[slot], w_sem.at[slot], WQR, R)
        _fetch(kt_hbm, c * R, sk - win, kv_buf.at[slot], kv_sem.at[slot], PR, PC)

    def fetch_v(c):
        slot = (c + NC) % NBUF
        _fetch(vt_hbm, c * R, sk - win, kv_buf.at[slot], kv_sem.at[slot], PR, PC)
        _fetch(wo_hbm, c * R, 0, wo_buf.at[slot], w_sem.at[slot], WOR, d)

    def head_mask(c):
        row = jax.lax.broadcasted_iota(jnp.int32, (G, R), 0) * DH
        col = jax.lax.broadcasted_iota(jnp.int32, (G, R), 1) + (c % CPG) * R
        return (col >= row) & (col < row + DH)

    x_cp = pltpu.make_async_copy(x_hbm, x_buf, x_sem.at[0])
    wr_cp = pltpu.make_async_copy(wr_hbm, wr_buf, x_sem.at[1])
    x_cp.start()
    wr_cp.start()
    fetch_k(0)
    x_cp.wait()
    wr_cp.wait()
    x = x_buf[...].astype(jnp.float32)
    xn = _rows8(_layernorm(x))
    s_scr[...] = jnp.zeros_like(s_scr)
    a_scr[...] = jnp.zeros_like(a_scr)

    def k_step(c, _):
        @pl.when(c + 1 < NC)
        def _():
            fetch_k(c + 1)

        @pl.when(c + 1 == NC)
        def _():
            fetch_v(0)

        slot = c % NBUF
        _wait(wq_buf.at[slot], w_sem.at[slot])
        _wait(kv_buf.at[slot], kv_sem.at[slot])
        q = jnp.where(head_mask(c), _dot(xn, wq_buf[slot]), 0.0).astype(jnp.bfloat16)
        s_scr[...] += _dot(q, kv_buf[slot])

        @pl.when(c % CPG == CPG - 1)
        def _():
            s = s_scr[...] * (DH ** -0.5)
            e = jnp.exp(s - jnp.max(s, axis=-1, keepdims=True))
            p = e / jnp.sum(e, axis=-1, keepdims=True)
            p_scr[c // CPG] = p.astype(jnp.bfloat16)
            s_scr[...] = jnp.zeros_like(s_scr)

    jax.lax.fori_loop(0, NC, k_step, None)

    def v_step(c, _):
        @pl.when(c + 1 < NC)
        def _():
            fetch_v(c + 1)

        @pl.when(c + 1 == NC)
        def _():
            _fetch(wg_hbm, 0, 0, wg_buf, x_sem.at[0], WGR, f // 4)

        slot = (c + NC) % NBUF
        _wait(kv_buf.at[slot], kv_sem.at[slot])
        _wait(wo_buf.at[slot], w_sem.at[slot])
        o = jax.lax.dot_general(p_scr[c // CPG], kv_buf[slot], (((1,), (1,)), ((), ())),
                                preferred_element_type=jnp.float32)
        o = jnp.where(head_mask(c), o, 0.0).astype(jnp.bfloat16)
        a_scr[...] += _dot(o, wo_buf[slot])

    jax.lax.fori_loop(0, NC, v_step, None)

    h = x + jnp.sum(a_scr[...], axis=0, keepdims=True)
    hn = _layernorm(h).astype(jnp.bfloat16).astype(jnp.float32)
    r = jnp.sum(hn * wr_buf[...].astype(jnp.float32).reshape(1, d), axis=-1, keepdims=True)
    hn8 = _rows8(hn)

    _fetch(wu_hbm, 0, 0, wu_buf, x_sem.at[1], WGR, f // 4)
    _wait(wg_buf, x_sem.at[0])
    gate = _dot(hn8, wg_buf[...])
    for i in range(ND):
        _fetch(wd_hbm, i * fc, 0, wd_buf.at[i], wd_sem.at[i], WOR, d)
        if i == 2:
            _wait(wu_buf, x_sem.at[1])
            up = _dot(hn8, wu_buf[...])
            act = (gate * jax.nn.sigmoid(gate) * up).astype(jnp.bfloat16)
    y = None
    for i in range(ND):
        _wait(wd_buf.at[i], wd_sem.at[i])
        t = _dot(act[:, i * fc:(i + 1) * fc], wd_buf[i])
        y = t if y is None else y + t
    y = y[0:1] * jax.nn.sigmoid(r)
    o_ref[...] = (h + (hn + (hn * 0.0 + y))).astype(o_ref.dtype)


@jax.jit
def pallas_sequential_preLN__sliding_block_cached__moe_arch_mod__decode_kernel(
    A_x: jax.Array,
    A_k_cache: jax.Array,
    A_v_cache: jax.Array,
    A_wq: jax.Array,
    A_wo: jax.Array,
    B_x: jax.Array,
    B_w_r: jax.Array,
    B_w_gate: jax.Array,
    B_w_up: jax.Array,
    B_w_down: jax.Array,
):
    del B_x
    d = A_x.shape[-1]
    sk = A_k_cache.shape[2]
    f = B_w_gate.shape[1]
    win = min(4096, max(256, sk // 4))
    kt = jnp.swapaxes(A_k_cache, 2, 3).reshape(HQ * DH, sk)
    vt = jnp.swapaxes(A_v_cache, 2, 3).reshape(HQ * DH, sk)
    bf = jnp.bfloat16
    out = pl.pallas_call(
        _kernel,
        out_shape=jax.ShapeDtypeStruct((1, d), A_x.dtype),
        in_specs=[pl.BlockSpec(memory_space=pl.ANY)] * 9,
        out_specs=pl.BlockSpec(memory_space=pltpu.VMEM),
        scratch_shapes=[
            pltpu.VMEM((NBUF, R, win), bf),
            pltpu.VMEM((NBUF, d, R), bf),
            pltpu.VMEM((NBUF, R, d), bf),
            pltpu.VMEM((d, f), bf),
            pltpu.VMEM((d, f), bf),
            pltpu.VMEM((ND, f // ND, d), bf),
            pltpu.VMEM((1, d), bf),
            pltpu.VMEM((d,), bf),
            pltpu.VMEM((G, win), jnp.float32),
            pltpu.VMEM((HQ // G, G, win), bf),
            pltpu.VMEM((G, d), jnp.float32),
            pltpu.SemaphoreType.DMA((NBUF,)),
            pltpu.SemaphoreType.DMA((NBUF,)),
            pltpu.SemaphoreType.DMA((2,)),
            pltpu.SemaphoreType.DMA((ND,)),
        ],
        compiler_params=pltpu.CompilerParams(vmem_limit_bytes=64 * 2**20),
    )(A_x.reshape(1, d), kt, vt, A_wq, A_wo, B_w_r, B_w_gate, B_w_up, B_w_down)
    return out.reshape(A_x.shape)
```
